```python
import os as _os
_os.environ.setdefault("JAX_PLATFORMS", "cpu")
import jax
import jax.numpy as jnp

def _softmax(x, axis=-1):
    return jax.nn.softmax(x, axis=axis)
def _gelu(x):
    return jax.nn.gelu(x, approximate=True)
def _silu(x):
    return jax.nn.silu(x)
def _sigmoid(x):
    return jax.nn.sigmoid(x)
def _layernorm(x, axis=-1, eps=1e-5):
    m = jnp.mean(x, axis=axis, keepdims=True)
    v = jnp.var(x, axis=axis, keepdims=True)
    return (x - m) / jnp.sqrt(v + eps)
def _scatter_add(tgt, idx, src, axis=0):
    return tgt.at[idx].add(src)
def _segment_sum(src, seg, n):
    return jax.ops.segment_sum(src, seg, n)
class _Rng:
    def __init__(self, key):
        self._k = key
    def _next(self):
        self._k, sub = jax.random.split(self._k)
        return sub
    def normal(self, shape):
        return jax.random.normal(self._next(), shape, dtype=jnp.bfloat16)
    def randint(self, lo, hi, shape):
        return jax.random.randint(self._next(), shape, lo, hi, dtype=jnp.int32)
    def uniform(self, shape, lo=0.0, hi=1.0):
        return jax.random.uniform(self._next(), shape, jnp.bfloat16, lo, hi)
    def permutation(self, n):
        return jax.random.permutation(self._next(), n)


kernel_name = 'standalone__instancenorm__sampling'

def setup_inputs():
    _rng = _Rng(jax.random.key(int.from_bytes(__import__("os").urandom(4), "little")))
    _w = (lambda a: (lambda t: t.astype(jnp.bfloat16) if jnp.issubdtype(t.dtype, jnp.floating) else t)(jnp.asarray(a)))
    B, C, H, W = 16, 640, 16, 32
    return {
        "x": _w((lambda *s: _rng.normal(s) * 0.05)(B, C, H, W)),
        "g": _w((lambda *s: _rng.normal(s) * 0.05)(C) + 1.0),
        "b": _w((lambda *s: _rng.normal(s) * 0.05)(C)),
    }

def reference(x, g, b):
    mu = x.mean(axis=(-2, -1), keepdims=True)
    var = ((x - mu) * (x - mu)).mean(axis=(-2, -1), keepdims=True)
    xhat = (x - mu) / jnp.sqrt(var + 1e-5)
    return xhat * g.reshape(1, -1, 1, 1) + b.reshape(1, -1, 1, 1)
```

```python
import jax
import jax.numpy as jnp
import jax.experimental.pallas as pl
import jax.experimental.pallas.tpu as pltpu


def _kernel(x_ref, g_ref, b_ref, o_ref):
    x = x_ref[...].astype(jnp.float32)
    n = x.shape[0]
    mu = jnp.sum(x, axis=0, keepdims=True) * (1.0 / n)
    d = x - mu
    var = jnp.sum(d * d, axis=0, keepdims=True) * (1.0 / n)
    scale = g_ref[...].astype(jnp.float32) / jnp.sqrt(var + 1e-5)
    o_ref[...] = (d * scale + b_ref[...].astype(jnp.float32)).astype(o_ref.dtype)


@jax.jit
def pallas_standalone__instancenorm__sampling_kernel(
    x: jax.Array,
    g: jax.Array,
    b: jax.Array,
):
    B, C, H, W = x.shape
    HW = H * W
    xt = x.transpose(0, 2, 3, 1).reshape(B, HW, C)
    g2 = g.reshape(1, C)
    b2 = b.reshape(1, C)
    out = pl.pallas_call(
        _kernel,
        grid=(B,),
        in_specs=[
            pl.BlockSpec((None, HW, C), lambda i: (i, 0, 0)),
            pl.BlockSpec((1, C), lambda i: (0, 0)),
            pl.BlockSpec((1, C), lambda i: (0, 0)),
        ],
        out_specs=pl.BlockSpec((None, HW, C), lambda i: (i, 0, 0)),
        out_shape=jax.ShapeDtypeStruct((B, HW, C), x.dtype),
        compiler_params=pltpu.CompilerParams(
            dimension_semantics=("parallel",),
        ),
    )(xt, g2, b2)
    return out.reshape(B, H, W, C).transpose(0, 3, 1, 2)
```

```python
import jax
import jax.numpy as jnp
import jax.experimental.pallas as pl
import jax.experimental.pallas.tpu as pltpu

_EPS = 1e-5
_DEPTH = 2
_K = 4
_WROWS = 32
_OVERLAP = 2


def _make_kernel(B, HW, C):
    K = _K
    Q = B // K
    D = _DEPTH
    S = B - _OVERLAP
    rows = _WROWS

    def kernel(x_hbm, g_hbm, b_hbm, o_hbm, buf, gbuf, bbuf, sem_in, sem_gb, sem_out):
        def rd(i):
            return pltpu.make_async_copy(
                x_hbm.at[i // Q, i % Q], buf.at[i // Q, i % Q], sem_in.at[i % D])

        cg = pltpu.make_async_copy(g_hbm, gbuf, sem_gb)
        cb = pltpu.make_async_copy(b_hbm, bbuf, sem_gb)
        cg.start()
        cb.start()
        for i in range(D):
            rd(i).start()
        cg.wait()
        cb.wait()
        g = gbuf[...].astype(jnp.float32).reshape(1, C)
        b = bbuf[...].astype(jnp.float32).reshape(1, C)

        def compute(i):
            x = buf[i // Q, i % Q].astype(jnp.float32)
            mu = jnp.sum(x, axis=0, keepdims=True) * (1.0 / HW)
            d = x - mu
            var = jnp.sum(d * d, axis=0, keepdims=True) * (1.0 / HW)
            scale = g / jnp.sqrt(var + _EPS)
            buf[i // Q, i % Q] = (d * scale + b).astype(buf.dtype)

        def body(i, carry):
            rd(i).wait()

            @pl.when(i + D < B)
            def _():
                rd(i + D).start()

            compute(i)
            return carry

        jax.lax.fori_loop(0, S, body, 0)

        outs = []
        state = {"done": S, "next_q": 0}

        def flush():
            while state["next_q"] < Q and (K - 1) * Q + state["next_q"] < state["done"]:
                q = state["next_q"]
                for j in range(HW // rows):
                    sl = (slice(None), q, pl.ds(j * rows, rows), slice(None))
                    w = pltpu.make_async_copy(buf.at[sl], o_hbm.at[sl], sem_out)
                    w.start()
                    outs.append(w)
                state["next_q"] = q + 1

        for i in range(S, B):
            rd(i).wait()
            if i + D < B:
                rd(i + D).start()
            flush()
            compute(i)
            state["done"] = i + 1
            flush()
        for w in outs:
            w.wait()

    return kernel


@jax.jit
def pallas_standalone__instancenorm__sampling_kernel(
    x: jax.Array,
    g: jax.Array,
    b: jax.Array,
):
    B, C, H, W = x.shape
    HW = H * W
    K = _K
    Q = B // K
    xt = x.transpose(0, 2, 3, 1).reshape(K, Q, HW, C)
    out = pl.pallas_call(
        _make_kernel(B, HW, C),
        in_specs=[
            pl.BlockSpec(memory_space=pl.ANY),
            pl.BlockSpec(memory_space=pl.ANY),
            pl.BlockSpec(memory_space=pl.ANY),
        ],
        out_specs=pl.BlockSpec(memory_space=pl.ANY),
        out_shape=jax.ShapeDtypeStruct((K, Q, HW, C), x.dtype),
        scratch_shapes=[
            pltpu.VMEM((K, Q, HW, C), x.dtype),
            pltpu.VMEM((C,), g.dtype),
            pltpu.VMEM((C,), b.dtype),
            pltpu.SemaphoreType.DMA((_DEPTH,)),
            pltpu.SemaphoreType.DMA(()),
            pltpu.SemaphoreType.DMA(()),
        ],
        compiler_params=pltpu.CompilerParams(vmem_limit_bytes=64 * 1024 * 1024),
    )(xt, g, b)
    return out.reshape(B, H, W, C).transpose(0, 3, 1, 2)
```

```python
import jax
import jax.numpy as jnp
import jax.experimental.pallas as pl
import jax.experimental.pallas.tpu as pltpu

_EPS = 1e-5
_K = 4
_RROWS = 16
_WROWS = 32
_TAIL = 176
_NPRE = 0
_RC = 64


def _make_kernel(B, HW, C, tail=_TAIL, npre=_NPRE):
    K = _K
    Q = B // K
    assert Q == 4 and HW % _RROWS == 0 and HW % _WROWS == 0 and HW % _RC == 0
    assert tail % _RROWS == 0 and 0 < tail < HW
    NJ = HW // _RROWS
    UPB = NJ // K
    NCH = HW // _RC
    TAIL_J = NJ - tail // _RROWS
    TAIL_SEM = 2

    def kernel(x_hbm, g_hbm, b_hbm, o_hbm, buf, gbuf, bbuf, sem_in, sem_out):
        def issue(q, j):
            if isinstance(q, int) and q == Q - 1:
                s = sem_in.at[jnp.where(j >= TAIL_J, TAIL_SEM, q % 2)]
            else:
                s = sem_in.at[q % 2]
            for r in range(K):
                sl = (r, q, pl.ds(pl.multiple_of(j * _RROWS, _RROWS), _RROWS))
                pltpu.make_async_copy(x_hbm.at[sl], buf.at[sl], s).start(priority=r % 2)

        def wait_in(q, start, size, sem_idx):
            sl = (slice(None), q, pl.ds(start, size))
            pltpu.make_async_copy(x_hbm.at[sl], buf.at[sl], sem_in.at[sem_idx]).wait()

        def write_group(q):
            for j in range(HW // _WROWS):
                sl = (slice(None), q, pl.ds(j * _WROWS, _WROWS))
                pltpu.make_async_copy(buf.at[sl], o_hbm.at[sl], sem_out).start()

        cg = pltpu.make_async_copy(g_hbm, gbuf, sem_out)
        cb = pltpu.make_async_copy(b_hbm, bbuf, sem_out)
        cg.start()
        cb.start()

        def issue_loop(u, c):
            issue(u // NJ, u % NJ)
            return c

        jax.lax.fori_loop(0, 2 * NJ, issue_loop, 0)
        cg.wait()
        cb.wait()
        g = gbuf[...].astype(jnp.float32).reshape(1, C)
        b = bbuf[...].astype(jnp.float32).reshape(1, C)

        def normalise(r, q, issue_q):
            points = [] if issue_q is None else [k * 3 * NCH // UPB for k in range(UPB)]
            step = [0]

            def tick():
                for k, pt in enumerate(points):
                    if pt == step[0]:
                        issue(issue_q, r * UPB + k)
                step[0] += 1

            xr = buf.at[r, q]
            acc = jnp.zeros((8, C), jnp.float32)
            for c in range(NCH):
                tick()
                x = xr[pl.ds(c * _RC, _RC), :].astype(jnp.float32)
                acc = acc + jnp.sum(x.reshape(_RC // 8, 8, C), axis=0)
            mu = jnp.sum(acc, axis=0, keepdims=True) * (1.0 / HW)
            acc = jnp.zeros((8, C), jnp.float32)
            for c in range(NCH):
                tick()
                d = xr[pl.ds(c * _RC, _RC), :].astype(jnp.float32) - mu
                acc = acc + jnp.sum((d * d).reshape(_RC // 8, 8, C), axis=0)
            var = jnp.sum(acc, axis=0, keepdims=True) * (1.0 / HW)
            scale = g / jnp.sqrt(var + _EPS)
            for c in range(NCH):
                tick()
                d = xr[pl.ds(c * _RC, _RC), :].astype(jnp.float32) - mu
                xr[pl.ds(c * _RC, _RC), :] = (d * scale + b).astype(buf.dtype)

        def normalise_range(q, r0, r1, issue_q=None):
            if r1 <= r0:
                return

            def body(r, c):
                normalise(r, q, issue_q)
                return c

            jax.lax.fori_loop(r0, r1, body, 0)

        wait_in(0, 0, HW, 0)
        normalise_range(0, 0, K, issue_q=2)
        wait_in(1, 0, HW, 1)
        normalise_range(1, 0, K, issue_q=3)
        wait_in(2, 0, HW, 0)
        normalise_range(2, 0, npre)
        wait_in(3, 0, HW - tail, 1)
        write_group(0)
        write_group(1)
        normalise_range(2, npre, K)
        write_group(2)
        wait_in(3, HW - tail, tail, TAIL_SEM)
        normalise_range(3, 0, K)
        write_group(3)
        pltpu.make_async_copy(buf, o_hbm, sem_out).wait()

    return kernel


def _build(x, g, b, **kw):
    B, C, H, W = x.shape
    HW = H * W
    K = _K
    Q = B // K
    xt = x.transpose(0, 2, 3, 1).reshape(K, Q, HW, C)
    out = pl.pallas_call(
        _make_kernel(B, HW, C, **kw),
        in_specs=[
            pl.BlockSpec(memory_space=pl.ANY),
            pl.BlockSpec(memory_space=pl.ANY),
            pl.BlockSpec(memory_space=pl.ANY),
        ],
        out_specs=pl.BlockSpec(memory_space=pl.ANY),
        out_shape=jax.ShapeDtypeStruct((K, Q, HW, C), x.dtype),
        scratch_shapes=[
            pltpu.VMEM((K, Q, HW, C), x.dtype),
            pltpu.VMEM((C,), g.dtype),
            pltpu.VMEM((C,), b.dtype),
            pltpu.SemaphoreType.DMA((3,)),
            pltpu.SemaphoreType.DMA(()),
        ],
        compiler_params=pltpu.CompilerParams(vmem_limit_bytes=64 * 1024 * 1024),
    )(xt, g, b)
    return out.reshape(B, H, W, C).transpose(0, 3, 1, 2)


@jax.jit
def pallas_standalone__instancenorm__sampling_kernel(
    x: jax.Array,
    g: jax.Array,
    b: jax.Array,
):
    return _build(x, g, b)
```
